```python
import os as _os
_os.environ.setdefault("JAX_PLATFORMS", "cpu")
import jax
import jax.numpy as jnp

def _softmax(x, axis=-1):
    return jax.nn.softmax(x, axis=axis)
def _gelu(x):
    return jax.nn.gelu(x, approximate=True)
def _silu(x):
    return jax.nn.silu(x)
def _sigmoid(x):
    return jax.nn.sigmoid(x)
def _layernorm(x, axis=-1, eps=1e-5):
    m = jnp.mean(x, axis=axis, keepdims=True)
    v = jnp.var(x, axis=axis, keepdims=True)
    return (x - m) / jnp.sqrt(v + eps)
def _scatter_add(tgt, idx, src, axis=0):
    return tgt.at[idx].add(src)
def _segment_sum(src, seg, n):
    return jax.ops.segment_sum(src, seg, n)
class _Rng:
    def __init__(self, key):
        self._k = key
    def _next(self):
        self._k, sub = jax.random.split(self._k)
        return sub
    def normal(self, shape):
        return jax.random.normal(self._next(), shape, dtype=jnp.bfloat16)
    def randint(self, lo, hi, shape):
        return jax.random.randint(self._next(), shape, lo, hi, dtype=jnp.int32)
    def uniform(self, shape, lo=0.0, hi=1.0):
        return jax.random.uniform(self._next(), shape, jnp.bfloat16, lo, hi)
    def permutation(self, n):
        return jax.random.permutation(self._next(), n)


kernel_name = 'sequential_preLN__mha_block__dense_activation_mish__prompt'

def setup_inputs():
    _rng = _Rng(jax.random.key(int.from_bytes(__import__("os").urandom(4), "little")))
    _w = (lambda a: (lambda t: t.astype(jnp.bfloat16) if jnp.issubdtype(t.dtype, jnp.floating) else t)(jnp.asarray(a)))
    def _A_setup():
        B, S, D, H = 1, 2048, 576, 32
        return {
            "x": _w((lambda *s: _rng.normal(s) * 0.05)(B, S, D)),
            "wqkv": _w((lambda *s: _rng.normal(s) * 0.05)(D, 3 * D)),
            "wo": _w((lambda *s: _rng.normal(s) * 0.05)(D, D)),
        }
    _A_in = _A_setup()

    def _B_setup():
        B, S, D, F = 1, 2048, 576, 4608
        return {
            "x": _w((lambda *s: _rng.normal(s) * 0.05)(B, S, D)),
            "w1": _w((lambda *s: _rng.normal(s) * 1.6)(D, F) * (D ** -0.5)),
            "b1": _w((lambda *s: _rng.normal(s) * 0.05)(F)),
            "w2": _w((lambda *s: _rng.normal(s) * 0.05)(F, D) * (F ** -0.5)),
        }
    _B_in = _B_setup()

    return {
        "A_x": _A_in["x"],
        "A_wqkv": _A_in["wqkv"],
        "A_wo": _A_in["wo"],
        "B_x": _B_in["x"],
        "B_w1": _B_in["w1"],
        "B_b1": _B_in["b1"],
        "B_w2": _B_in["w2"],
    }

def reference(A_x, A_wqkv, A_wo, B_x, B_w1, B_b1, B_w2):
    def _A_ref(x, wqkv, wo):
        B, S, D = x.shape
        H = 32
        Dh = D // H
        qkv = (lambda x, *d: x.transpose(*d))((x @ wqkv).reshape(B, S, 3, H, Dh), 2, 0, 3, 1, 4)
        q, k, v = qkv[0], qkv[1], qkv[2]
        scores = jnp.einsum("bhqd,bhkd->bhqk", q, k) * (Dh ** -0.5)
        p = _softmax(scores, axis=-1)
        o = jnp.einsum("bhqk,bhkd->bhqd", p, v)
        return (lambda x, *d: x.transpose(*d))(o, 0, 2, 1, 3).reshape(B, S, D) @ wo

    def _B_ref(x, w1, b1, w2):
        h = jnp.einsum("bsd,df->bsf", x, w1) + b1
        sp = jnp.log1p(jnp.exp(-jnp.abs(h))) + jnp.where(h > 0, h, jnp.zeros_like(h))
        act = h * jnp.tanh(sp)
        return jnp.einsum("bsf,fd->bsd", act, w2)

    x = A_x
    h = x + _A_ref(_layernorm(x, axis=-1), A_wqkv, A_wo)
    h2 = h + _B_ref(_layernorm(h, axis=-1), B_w1, B_b1, B_w2)
    return h2
```

```python
import functools

import jax
import jax.numpy as jnp
import jax.experimental.pallas as pl
import jax.experimental.pallas.tpu as pltpu

F32 = jnp.float32
BF16 = jnp.bfloat16

H = 32
DH = 18
HPT = 7
NT = 5
ONES_LANE = 126
LOG2E = 1.4426950408889634


def _layernorm(x, eps=1e-5):
    m = jnp.mean(x, axis=-1, keepdims=True)
    xc = x - m
    v = jnp.mean(xc * xc, axis=-1, keepdims=True)
    return xc * jax.lax.rsqrt(v + eps)


def _mish(h):
    sp = jnp.log1p(jnp.exp(-jnp.abs(h))) + jnp.where(h > 0, h, jnp.zeros_like(h))
    return h * jnp.tanh(sp)


def _kernel(x_ref, wqkv_ref, wo_ref, w1_ref, b1_ref, w2_ref, o_ref,
            q_s, k_s, v_s, oacc_s, *, S, D, F, TQ, RB, FC):
    i = pl.program_id(0)
    qscale = (DH ** -0.5) * LOG2E

    @pl.when(i == 0)
    def _():
        lane = jax.lax.broadcasted_iota(jnp.int32, (RB, 128), 1)

        def body(r, c):
            rows = pl.ds(pl.multiple_of(r * RB, RB), RB)
            xn = _layernorm(x_ref[rows, :].astype(F32)).astype(BF16)
            qkv = jnp.dot(xn, wqkv_ref[...], preferred_element_type=F32)
            for t in range(NT):
                q = qkv[:, t * 128:(t + 1) * 128] * qscale
                k = qkv[:, (NT + t) * 128:(NT + t + 1) * 128]
                v = qkv[:, (2 * NT + t) * 128:(2 * NT + t + 1) * 128]
                v = jnp.where(lane == ONES_LANE, 1.0, v)
                q_s[t, rows, :] = q.astype(BF16)
                k_s[t, rows, :] = k.astype(BF16)
                v_s[t, rows, :] = v.astype(BF16)
            return c

        jax.lax.fori_loop(0, S // RB, body, 0)

    qrows = pl.ds(pl.multiple_of(i * TQ, TQ), TQ)
    oacc_s[...] = jnp.zeros(oacc_s.shape, F32)
    lane_q = jax.lax.broadcasted_iota(jnp.int32, (TQ, 128), 1)

    def head_body(h, c):
        t = h // HPT
        j = h - t * HPT
        lo = j * DH
        mask = jnp.logical_and(lane_q >= lo, lane_q < lo + DH)
        q = jnp.where(mask, q_s[t, qrows, :], jnp.zeros((TQ, 128), BF16))
        s = jax.lax.dot_general(q, k_s[t], (((1,), (1,)), ((), ())),
                                preferred_element_type=F32)
        m = jnp.max(s, axis=-1, keepdims=True)
        p = jnp.exp2(s - m).astype(BF16)
        o = jnp.dot(p, v_s[t], preferred_element_type=F32)
        l = o[:, ONES_LANE:ONES_LANE + 1]
        oacc_s[t] = jnp.where(mask, o / l, oacc_s[t])
        return c

    jax.lax.fori_loop(0, H, head_body, 0)

    attn = jnp.zeros((TQ, D), F32)
    for t in range(NT):
        attn = attn + jnp.dot(oacc_s[t].astype(BF16), wo_ref[t],
                              preferred_element_type=F32)
    hres = x_ref[qrows, :].astype(F32) + attn
    hn = _layernorm(hres).astype(BF16)

    acc = hres
    for c in range(F // FC):
        a = jnp.dot(hn, w1_ref[:, c * FC:(c + 1) * FC], preferred_element_type=F32)
        a = a + b1_ref[:, c * FC:(c + 1) * FC].astype(F32)
        a = _mish(a).astype(BF16)
        acc = acc + jnp.dot(a, w2_ref[c * FC:(c + 1) * FC, :], preferred_element_type=F32)
    o_ref[...] = acc.astype(o_ref.dtype)


def _pack_heads_cols(w):
    din = w.shape[0]
    w = w.reshape(din, H, DH)
    w = jnp.pad(w, ((0, 0), (0, NT * HPT - H), (0, 0)))
    w = w.reshape(din, NT, HPT * DH)
    w = jnp.pad(w, ((0, 0), (0, 0), (0, 128 - HPT * DH)))
    return w.reshape(din, NT * 128)


@jax.jit
def pallas_sequential_preLN__mha_block__dense_activation_mish__prompt_kernel(
    A_x: jax.Array,
    A_wqkv: jax.Array,
    A_wo: jax.Array,
    B_x: jax.Array,
    B_w1: jax.Array,
    B_b1: jax.Array,
    B_w2: jax.Array,
):
    B, S, D = A_x.shape
    F = B_w1.shape[1]
    assert B == 1 and D == H * DH
    TQ, RB, FC = 256, 256, 512

    x = A_x.reshape(S, D)
    wq = _pack_heads_cols(A_wqkv[:, 0 * D:1 * D])
    wk = _pack_heads_cols(A_wqkv[:, 1 * D:2 * D])
    wv = _pack_heads_cols(A_wqkv[:, 2 * D:3 * D])
    wqkv = jnp.concatenate([wq, wk, wv], axis=1)
    wo = _pack_heads_cols(A_wo.T).T.reshape(NT, 128, D)
    b1 = B_b1.reshape(1, F)

    full = lambda shape: pl.BlockSpec(shape, lambda i: (0,) * len(shape))
    kernel = functools.partial(_kernel, S=S, D=D, F=F, TQ=TQ, RB=RB, FC=FC)
    out = pl.pallas_call(
        kernel,
        grid=(S // TQ,),
        in_specs=[
            full((S, D)),
            full((D, 3 * NT * 128)),
            full((NT, 128, D)),
            full((D, F)),
            full((1, F)),
            full((F, D)),
        ],
        out_specs=pl.BlockSpec((TQ, D), lambda i: (i, 0)),
        out_shape=jax.ShapeDtypeStruct((S, D), A_x.dtype),
        scratch_shapes=[
            pltpu.VMEM((NT, S, 128), BF16),
            pltpu.VMEM((NT, S, 128), BF16),
            pltpu.VMEM((NT, S, 128), BF16),
            pltpu.VMEM((NT, TQ, 128), F32),
        ],
        compiler_params=pltpu.CompilerParams(
            dimension_semantics=("arbitrary",),
            vmem_limit_bytes=100 * 1024 * 1024,
        ),
    )(x, wqkv, wo, B_w1, b1, B_w2)
    return out.reshape(B, S, D)
```

```python
import functools
import jax
import jax.numpy as jnp
import jax.experimental.pallas as pl
import jax.experimental.pallas.tpu as pltpu

F32 = jnp.float32
BF16 = jnp.bfloat16
H = 32; DH = 18; HPT = 7; NT = 5
GV = 32
GO = 24
LOG2E = 1.4426950408889634

def _ln_rows(x, eps=1e-5):
    m = jnp.mean(x, axis=-1, keepdims=True)
    xc = x - m
    v = jnp.mean(xc * xc, axis=-1, keepdims=True)
    return xc * jax.lax.rsqrt(v + eps)

def _ln_cols(x, eps=1e-5):
    m = jnp.mean(x, axis=0, keepdims=True)
    xc = x - m
    v = jnp.mean(xc * xc, axis=0, keepdims=True)
    return xc * jax.lax.rsqrt(v + eps)

def _mish(h):
    sp = jnp.log1p(jnp.exp(-jnp.abs(h))) + jnp.where(h > 0, h, jnp.zeros_like(h))
    return h * jnp.tanh(sp)

def _tile_width(t):
    return min(HPT * DH, H * DH - t * HPT * DH)

def _kernel(xT_hbm, wqkv_hbm, wo_hbm, w1_hbm, b1_hbm, w2T_hbm, oT_ref,
            xT, wqkv, wo, w1, b1, w2T, woT, q_s, k_s, vT_s, o_s, xsems, sems,
            *, S, D, F, TQ, RB, FC, UNROLL):
    i = pl.program_id(0)
    qscale = (DH ** -0.5) * LOG2E
    NR = S // RB
    xcopies = [pltpu.make_async_copy(xT_hbm.at[:, pl.ds(r * RB, RB)], xT.at[:, pl.ds(r * RB, RB)], xsems.at[r])
               for r in range(NR)]
    srcs = (wqkv_hbm, wo_hbm, w1_hbm, b1_hbm, w2T_hbm)
    dsts = (wqkv, wo, w1, b1, w2T)
    copies = [pltpu.make_async_copy(s, d, sems.at[n]) for n, (s, d) in enumerate(zip(srcs, dsts))]

    @pl.when(i == 0)
    def _():
        xcopies[0].start()
        copies[0].start()
        for c in xcopies[1:]:
            c.start()
        for c in copies[1:]:
            c.start()
        copies[0].wait()

        def tile(qkv, base, t):
            w = _tile_width(t)
            off = base + t * HPT * DH
            a = qkv[:, off:off + w]
            return jnp.concatenate([a, jnp.zeros((RB, 128 - w), F32)], axis=1)

        vpad = jnp.concatenate([jnp.ones((1, RB), F32), jnp.zeros((GV - DH - 1, RB), F32)], axis=0)

        def body(r, c):
            rows = pl.ds(pl.multiple_of(r * RB, RB), RB)
            pltpu.make_async_copy(xT_hbm.at[:, rows], xT.at[:, rows], xsems.at[r]).wait()
            x = xT[:, rows].astype(F32).T
            xn = _ln_rows(x).astype(BF16)
            qkv = jnp.dot(xn, wqkv[...], preferred_element_type=F32)
            for t in range(NT):
                q_s[t, rows, :] = (tile(qkv, 0, t) * qscale).astype(BF16)
                k_s[t, rows, :] = tile(qkv, D, t).astype(BF16)
            vT = qkv[:, 2 * D:3 * D].T
            for h in range(H):
                blk = jnp.concatenate([vT[h * DH:(h + 1) * DH, :], vpad], axis=0)
                vT_s[h, :, rows] = blk.astype(BF16)
            return c
        jax.lax.fori_loop(0, NR, body, 0)

        copies[1].wait()
        wot = wo[...].astype(F32).T
        zpad = jnp.zeros((D, GO - DH), F32)
        cols = []
        for h in range(H):
            cols += [wot[:, h * DH:(h + 1) * DH], zpad]
        woT[...] = jnp.concatenate(cols, axis=1).astype(BF16)

    qrows = pl.ds(pl.multiple_of(i * TQ, TQ), TQ)
    lane_q = jax.lax.broadcasted_iota(jnp.int32, (TQ, 128), 1)
    row_o = jax.lax.broadcasted_iota(jnp.int32, (GO, TQ), 0)

    def head_body(h, c):
        t = h // HPT
        lo = (h - t * HPT) * DH
        mask = jnp.logical_and(lane_q >= lo, lane_q < lo + DH)
        q = jnp.where(mask, q_s[t, qrows, :], jnp.zeros((TQ, 128), BF16))
        sc = jax.lax.dot_general(q, k_s[t], (((1,), (1,)), ((), ())),
                                 preferred_element_type=F32)
        m = jnp.max(sc, axis=-1, keepdims=True)
        p = jnp.exp2(sc - m).astype(BF16)
        oT = jax.lax.dot_general(vT_s[h], p, (((1,), (1,)), ((), ())),
                                 preferred_element_type=F32)
        l = oT[DH:DH + 1, :]
        o_s[h] = jnp.where(row_o < DH, oT[:GO, :] / l, 0.0)
        return c

    jax.lax.fori_loop(0, H, head_body, 0, unroll=UNROLL)

    @pl.when(i == 0)
    def _():
        for c in copies[2:]:
            c.wait()

    oall = o_s[...].reshape(H * GO, TQ).astype(BF16)
    hT = xT[:, qrows].astype(F32) + jnp.dot(woT[...], oall, preferred_element_type=F32)
    hn = _ln_cols(hT).T.astype(BF16)

    acc = hT
    for c in range(F // FC):
        a = jnp.dot(hn, w1[:, c * FC:(c + 1) * FC], preferred_element_type=F32)
        a = a + b1[:, c * FC:(c + 1) * FC].astype(F32)
        a = _mish(a).astype(BF16)
        acc = acc + jax.lax.dot_general(w2T[:, c * FC:(c + 1) * FC], a, (((1,), (1,)), ((), ())),
                                        preferred_element_type=F32)
    oT_ref[...] = acc.astype(oT_ref.dtype)


@jax.jit
def pallas_sequential_preLN__mha_block__dense_activation_mish__prompt_kernel(
    A_x, A_wqkv, A_wo, B_x, B_w1, B_b1, B_w2):
    B, S, D = A_x.shape
    F = B_w1.shape[1]
    TQ, RB, FC, UNROLL = 512, 256, 512, 4
    xT = A_x.reshape(S, D).T
    w2T = B_w2.T
    b1 = B_b1.reshape(1, F)
    hbm = pl.BlockSpec(memory_space=pl.ANY)
    kernel = functools.partial(_kernel, S=S, D=D, F=F, TQ=TQ, RB=RB, FC=FC, UNROLL=UNROLL)
    outT = pl.pallas_call(
        kernel,
        grid=(S // TQ,),
        in_specs=[hbm] * 6,
        out_specs=pl.BlockSpec((D, TQ), lambda i: (0, i)),
        out_shape=jax.ShapeDtypeStruct((D, S), A_x.dtype),
        scratch_shapes=[
            pltpu.VMEM((D, S), BF16),
            pltpu.VMEM((D, 3 * D), BF16),
            pltpu.VMEM((D, D), BF16),
            pltpu.VMEM((D, F), BF16),
            pltpu.VMEM((1, F), BF16),
            pltpu.VMEM((D, F), BF16),
            pltpu.VMEM((D, H * GO), BF16),
            pltpu.VMEM((NT, S, 128), BF16),
            pltpu.VMEM((NT, S, 128), BF16),
            pltpu.VMEM((H, GV, S), BF16),
            pltpu.VMEM((H, GO, TQ), F32),
            pltpu.SemaphoreType.DMA((S // RB,)),
            pltpu.SemaphoreType.DMA((5,)),
        ],
        compiler_params=pltpu.CompilerParams(
            dimension_semantics=("arbitrary",),
            vmem_limit_bytes=100 * 1024 * 1024,
        ),
    )(xT, A_wqkv, A_wo, B_w1, b1, w2T)
    return outT.T.reshape(B, S, D)
```

```python
import functools

import jax
import jax.numpy as jnp
import jax.experimental.pallas as pl
import jax.experimental.pallas.tpu as pltpu

F32 = jnp.float32
BF16 = jnp.bfloat16
H = 32
DH = 18
HPT = 7
NT = 5
GV = 32
GO = 24
LOG2E = 1.4426950408889634


def _ln_rows(x, eps=1e-5):
    m = jnp.mean(x, axis=-1, keepdims=True)
    xc = x - m
    v = jnp.mean(xc * xc, axis=-1, keepdims=True)
    return xc * jax.lax.rsqrt(v + eps)


def _ln_cols(x, eps=1e-5):
    m = jnp.mean(x, axis=0, keepdims=True)
    xc = x - m
    v = jnp.mean(xc * xc, axis=0, keepdims=True)
    return xc * jax.lax.rsqrt(v + eps)


def _mish(h):
    sp = jnp.log1p(jnp.exp(-jnp.abs(h))) + jnp.where(h > 0, h, jnp.zeros_like(h))
    return h * jnp.tanh(sp)


def _tile_width(t):
    return min(HPT * DH, H * DH - t * HPT * DH)


def _kernel(xT_hbm, wqkv_hbm, wo_hbm, w1_hbm, b1_hbm, w2T_hbm, oT_ref,
            xT, wqkv, wo, w1, b1, w2T, woT, q_s, k_s, vT_s, o_s, xsems, sems,
            *, S, D, F, TQ, RB, FC, UNROLL):
    i = pl.program_id(0)
    qscale = (DH ** -0.5) * LOG2E
    NR = S // RB
    xcopies = [pltpu.make_async_copy(xT_hbm.at[:, pl.ds(r * RB, RB)],
                                     xT.at[:, pl.ds(r * RB, RB)], xsems.at[r])
               for r in range(NR)]
    srcs = (wqkv_hbm, wo_hbm, w1_hbm, b1_hbm, w2T_hbm)
    dsts = (wqkv, wo, w1, b1, w2T)
    copies = [pltpu.make_async_copy(s, d, sems.at[n])
              for n, (s, d) in enumerate(zip(srcs, dsts))]

    @pl.when(i == 0)
    def _():
        xcopies[0].start()
        copies[0].start()
        for c in xcopies[1:]:
            c.start()
        for c in copies[1:]:
            c.start()
        copies[0].wait()

        def tile(qkv, base, t):
            w = _tile_width(t)
            off = base + t * HPT * DH
            a = qkv[:, off:off + w]
            return jnp.concatenate([a, jnp.zeros((RB, 128 - w), F32)], axis=1)

        vpad = jnp.concatenate([jnp.ones((1, RB), F32),
                                jnp.zeros((GV - DH - 1, RB), F32)], axis=0)

        def body(r, c):
            rows = pl.ds(pl.multiple_of(r * RB, RB), RB)
            pltpu.make_async_copy(xT_hbm.at[:, rows], xT.at[:, rows], xsems.at[r]).wait()
            x = xT[:, rows].astype(F32).T
            xn = _ln_rows(x).astype(BF16)
            qkv = jnp.dot(xn, wqkv[...], preferred_element_type=F32)
            for t in range(NT):
                q_s[t, rows, :] = (tile(qkv, 0, t) * qscale).astype(BF16)
                k_s[t, rows, :] = tile(qkv, D, t).astype(BF16)
            vT = qkv[:, 2 * D:3 * D].T
            for h in range(H):
                blk = jnp.concatenate([vT[h * DH:(h + 1) * DH, :], vpad], axis=0)
                vT_s[h, :, rows] = blk.astype(BF16)
            return c

        jax.lax.fori_loop(0, NR, body, 0)

        copies[1].wait()
        wot = wo[...].astype(F32).T
        zpad = jnp.zeros((D, GO - DH), F32)
        cols = []
        for h in range(H):
            cols += [wot[:, h * DH:(h + 1) * DH], zpad]
        woT[...] = jnp.concatenate(cols, axis=1).astype(BF16)

    qrows = pl.ds(pl.multiple_of(i * TQ, TQ), TQ)
    lane_q = jax.lax.broadcasted_iota(jnp.int32, (TQ, 128), 1)
    row_o = jax.lax.broadcasted_iota(jnp.int32, (GO, TQ), 0)

    def head_body(h, c):
        t = h // HPT
        lo = (h - t * HPT) * DH
        mask = jnp.logical_and(lane_q >= lo, lane_q < lo + DH)
        q = jnp.where(mask, q_s[t, qrows, :], jnp.zeros((TQ, 128), BF16))
        sc = jax.lax.dot_general(q, k_s[t], (((1,), (1,)), ((), ())),
                                 preferred_element_type=F32)
        m = jnp.max(sc, axis=-1, keepdims=True)
        p = jnp.exp2(sc - m).astype(BF16)
        oT = jax.lax.dot_general(vT_s[h], p, (((1,), (1,)), ((), ())),
                                 preferred_element_type=F32)
        l = oT[DH:DH + 1, :]
        o_s[h] = jnp.where(row_o < DH, oT[:GO, :] / l, 0.0)
        return c

    jax.lax.fori_loop(0, H, head_body, 0, unroll=UNROLL)

    @pl.when(i == 0)
    def _():
        for c in copies[2:]:
            c.wait()

    oall = o_s[...].reshape(H * GO, TQ).astype(BF16)
    hT = xT[:, qrows].astype(F32) + jnp.dot(woT[...], oall, preferred_element_type=F32)
    hn = _ln_cols(hT).T.astype(BF16)

    acc = hT
    for c in range(F // FC):
        a = jnp.dot(hn, w1[:, c * FC:(c + 1) * FC], preferred_element_type=F32)
        a = a + b1[:, c * FC:(c + 1) * FC].astype(F32)
        a = _mish(a).astype(BF16)
        acc = acc + jax.lax.dot_general(w2T[:, c * FC:(c + 1) * FC], a,
                                        (((1,), (1,)), ((), ())),
                                        preferred_element_type=F32)
    oT_ref[...] = acc.astype(oT_ref.dtype)


@jax.jit
def pallas_sequential_preLN__mha_block__dense_activation_mish__prompt_kernel(
    A_x: jax.Array,
    A_wqkv: jax.Array,
    A_wo: jax.Array,
    B_x: jax.Array,
    B_w1: jax.Array,
    B_b1: jax.Array,
    B_w2: jax.Array,
):
    B, S, D = A_x.shape
    F = B_w1.shape[1]
    assert B == 1 and D == H * DH
    TQ, RB, FC, UNROLL = 512, 256, 512, 4
    xT = A_x.reshape(S, D).T
    w2T = B_w2.T
    b1 = B_b1.reshape(1, F)
    hbm = pl.BlockSpec(memory_space=pl.ANY)
    kernel = functools.partial(_kernel, S=S, D=D, F=F, TQ=TQ, RB=RB, FC=FC, UNROLL=UNROLL)
    outT = pl.pallas_call(
        kernel,
        grid=(S // TQ,),
        in_specs=[hbm] * 6,
        out_specs=pl.BlockSpec((D, TQ), lambda i: (0, i)),
        out_shape=jax.ShapeDtypeStruct((D, S), A_x.dtype),
        scratch_shapes=[
            pltpu.VMEM((D, S), BF16),
            pltpu.VMEM((D, 3 * D), BF16),
            pltpu.VMEM((D, D), BF16),
            pltpu.VMEM((D, F), BF16),
            pltpu.VMEM((1, F), BF16),
            pltpu.VMEM((D, F), BF16),
            pltpu.VMEM((D, H * GO), BF16),
            pltpu.VMEM((NT, S, 128), BF16),
            pltpu.VMEM((NT, S, 128), BF16),
            pltpu.VMEM((H, GV, S), BF16),
            pltpu.VMEM((H, GO, TQ), F32),
            pltpu.SemaphoreType.DMA((S // RB,)),
            pltpu.SemaphoreType.DMA((5,)),
        ],
        compiler_params=pltpu.CompilerParams(
            dimension_semantics=("arbitrary",),
            vmem_limit_bytes=100 * 1024 * 1024,
        ),
    )(xT, A_wqkv, A_wo, B_w1, b1, w2T)
    return outT.T.reshape(B, S, D)
```
